```python
import os as _os
_os.environ.setdefault("JAX_PLATFORMS", "cpu")
import jax
import jax.numpy as jnp

def _softmax(x, axis=-1):
    return jax.nn.softmax(x, axis=axis)
def _gelu(x):
    return jax.nn.gelu(x, approximate=True)
def _silu(x):
    return jax.nn.silu(x)
def _sigmoid(x):
    return jax.nn.sigmoid(x)
def _layernorm(x, axis=-1, eps=1e-5):
    m = jnp.mean(x, axis=axis, keepdims=True)
    v = jnp.var(x, axis=axis, keepdims=True)
    return (x - m) / jnp.sqrt(v + eps)
def _scatter_add(tgt, idx, src, axis=0):
    return tgt.at[idx].add(src)
def _segment_sum(src, seg, n):
    return jax.ops.segment_sum(src, seg, n)
class _Rng:
    def __init__(self, key):
        self._k = key
    def _next(self):
        self._k, sub = jax.random.split(self._k)
        return sub
    def normal(self, shape):
        return jax.random.normal(self._next(), shape, dtype=jnp.bfloat16)
    def randint(self, lo, hi, shape):
        return jax.random.randint(self._next(), shape, lo, hi, dtype=jnp.int32)
    def uniform(self, shape, lo=0.0, hi=1.0):
        return jax.random.uniform(self._next(), shape, jnp.bfloat16, lo, hi)
    def permutation(self, n):
        return jax.random.permutation(self._next(), n)


kernel_name = 'standalone__gqa_block_cached__near_ridge'

def setup_inputs():
    _rng = _Rng(jax.random.key(int.from_bytes(__import__("os").urandom(4), "little")))
    _w = (lambda a: (lambda t: t.astype(jnp.bfloat16) if jnp.issubdtype(t.dtype, jnp.floating) else t)(jnp.asarray(a)))
    B, Sq, D = 16, 128, 576
    Hq, Hkv, Sk, Dh = 32, 16, 1024, 128
    assert Hq % Hkv == 0, (Hq, Hkv)
    return {
        "x": _w((lambda *s: _rng.normal(s) * 0.8)(B, Sq, D)),
        "k_cache": _w((lambda *s: _rng.normal(s) * 0.8)(B, Hkv, Sk, Dh)),
        "v_cache": _w((lambda *s: _rng.normal(s) * 0.05)(B, Hkv, Sk, Dh)),
        "wq": _w((lambda *s: _rng.normal(s) * 0.8)(D, Hq * Dh) * (D ** -0.5)),
        "wo": _w((lambda *s: _rng.normal(s) * 0.05)(Hq * Dh, D) * ((Hq * Dh) ** -0.5)),
    }

def reference(x, k_cache, v_cache, wq, wo):
    B, Sq, D = x.shape
    Hq, Dh = 32, 128
    Hkv = k_cache.shape[1]
    rep = Hq // Hkv
    q = (lambda x, *d: x.transpose(*d))((x @ wq).reshape(B, Sq, Hq, Dh), 0, 2, 1, 3)
    k = jnp.repeat(k_cache, rep, axis=1)
    v = jnp.repeat(v_cache, rep, axis=1)
    scores = jnp.einsum("bhqd,bhkd->bhqk", q, k) * (Dh ** -0.5)
    p = _softmax(scores, axis=-1)
    o = jnp.einsum("bhqk,bhkd->bhqd", p, v)
    return (lambda x, *d: x.transpose(*d))(o, 0, 2, 1, 3).reshape(B, Sq, Hq * Dh) @ wo
```

```python
import functools

import jax
import jax.numpy as jnp
import jax.experimental.pallas as pl
import jax.experimental.pallas.tpu as pltpu

HQ = 32
DH = 128
HB = 4


def _kernel(xt_ref, k_ref, v_ref, wq_ref, wot_ref, o_ref, q_sc, att_sc, *, hb, rep, scale):
    j = pl.program_id(1)
    nj = pl.num_programs(1)
    sq = q_sc.shape[1] // rep

    @pl.when(j == 0)
    def _():
        q = jax.lax.dot_general(xt_ref[...], wq_ref[...], (((0,), (0,)), ((), ())),
                                preferred_element_type=jnp.float32)
        q = (q * scale).astype(q_sc.dtype)
        for h in range(HQ):
            q_sc[h // rep, pl.ds((h % rep) * sq, sq), :] = q[:, h * DH:(h + 1) * DH]

    for h in range(hb):
        kv = j * hb + h
        k = k_ref[h]
        v = v_ref[h]
        q = q_sc[kv]
        s = jax.lax.dot_general(q, k, (((1,), (1,)), ((), ())),
                                preferred_element_type=jnp.float32)
        m = jnp.max(s, axis=-1, keepdims=True)
        p = jnp.exp(s - m)
        l = jnp.sum(p, axis=-1, keepdims=True)
        o = jnp.dot(p.astype(v.dtype), v, preferred_element_type=jnp.float32)
        o = (o / l).astype(att_sc.dtype)
        for r in range(rep):
            col = pl.multiple_of((kv * rep + r) * DH, DH)
            att_sc[:, pl.ds(col, DH)] = o[r * sq:(r + 1) * sq]

    @pl.when(j == nj - 1)
    def _():
        o_ref[...] = jax.lax.dot_general(
            wot_ref[...], att_sc[...], (((1,), (1,)), ((), ())),
            preferred_element_type=jnp.float32).astype(o_ref.dtype)


@jax.jit
def pallas_standalone__gqa_block_cached__near_ridge_kernel(
    x: jax.Array,
    k_cache: jax.Array,
    v_cache: jax.Array,
    wq: jax.Array,
    wo: jax.Array,
):
    B, Sq, D = x.shape
    _, Hkv, Sk, Dh = k_cache.shape
    rep = HQ // Hkv
    hb = HB
    scale = float(DH) ** -0.5
    grid = (B, Hkv // hb)
    xt = x.transpose(0, 2, 1)
    wot = wo.T
    out_t = pl.pallas_call(
        functools.partial(_kernel, hb=hb, rep=rep, scale=scale),
        grid=grid,
        in_specs=[
            pl.BlockSpec((None, D, Sq), lambda b, j: (b, 0, 0)),
            pl.BlockSpec((None, hb, Sk, Dh), lambda b, j: (b, j, 0, 0)),
            pl.BlockSpec((None, hb, Sk, Dh), lambda b, j: (b, j, 0, 0)),
            pl.BlockSpec((D, HQ * DH), lambda b, j: (0, 0)),
            pl.BlockSpec((D, HQ * DH), lambda b, j: (0, 0)),
        ],
        out_specs=pl.BlockSpec((None, D, Sq), lambda b, j: (b, 0, 0)),
        out_shape=jax.ShapeDtypeStruct((B, D, Sq), x.dtype),
        scratch_shapes=[
            pltpu.VMEM((Hkv, rep * Sq, DH), jnp.bfloat16),
            pltpu.VMEM((Sq, HQ * DH), jnp.bfloat16),
        ],
        compiler_params=pltpu.CompilerParams(
            dimension_semantics=("arbitrary", "arbitrary"),
            vmem_limit_bytes=96 * 1024 * 1024,
        ),
    )(xt, k_cache, v_cache, wq, wot)
    return out_t.transpose(0, 2, 1)
```

```python
import functools

import jax
import jax.numpy as jnp
import jax.experimental.pallas as pl
import jax.experimental.pallas.tpu as pltpu

HQ = 32
DH = 128
HB = 8
RC = 32


def _kernel(x0_ref, xn_ref, k_ref, v_ref, wq_hbm, wot_hbm, o_ref,
            wq_sc, wo_sc, q_sc, p0_sc, p1_sc, r0_sc, r1_sc, a0_sc, a1_sc, acc_sc, sem_q, sem_o,
            *, hb, rep, nj, nb, scale):
    t = pl.program_id(0)
    nt = nb * nj
    b = t // nj
    j = t % nj
    sq = x0_ref.shape[1]
    cw = hb * rep * DH
    nh = hb * rep
    p_sc = (p0_sc, p1_sc)
    r_sc = (r0_sc, r1_sc)
    a_sc = (a0_sc, a1_sc)

    def wq_copy(c):
        return pltpu.make_async_copy(wq_hbm.at[:, pl.ds(c * cw, cw)], wq_sc.at[c], sem_q.at[c])

    def wo_copy(c):
        return pltpu.make_async_copy(wot_hbm.at[:, pl.ds(c * cw, cw)], wo_sc.at[c], sem_o.at[c])

    def qproj(x_ref, c, slot):
        q = jax.lax.dot_general(x_ref[...], wq_sc[c], (((0,), (0,)), ((), ())),
                                preferred_element_type=jnp.float32)
        q = (q * scale).astype(q_sc.dtype)
        for h in range(nh):
            q_sc[slot, c * hb + h // rep, pl.ds((h % rep) * sq, sq), :] = q[:, h * DH:(h + 1) * DH]

    def qk(h):
        return jax.lax.dot_general(q_sc[b % 2, j * hb + h], k_ref[h], (((1,), (1,)), ((), ())),
                                   preferred_element_type=jnp.float32)

    def softmax(h, s, par):
        for c in range(0, rep * sq, RC):
            sc = s[c:c + RC]
            m = jnp.max(sc, axis=-1, keepdims=True)
            p = jnp.exp2(sc - m)
            r_sc[par][h, c:c + RC, :] = 1.0 / jnp.sum(p, axis=-1, keepdims=True)
            p_sc[par][h, c:c + RC, :] = p.astype(jnp.bfloat16)

    def pv(h, par):
        o = jnp.dot(p_sc[par][h], v_ref[h], preferred_element_type=jnp.float32)
        o = (o * r_sc[par][h]).astype(jnp.bfloat16)
        for rr in range(rep):
            a_sc[par][:, (h * rep + rr) * DH:(h * rep + rr + 1) * DH] = o[rr * sq:(rr + 1) * sq]

    def outproj(par):
        c = (t - 2) % nj
        part = jax.lax.dot_general(wo_sc[c], a_sc[par][...], (((1,), (1,)), ((), ())),
                                   preferred_element_type=jnp.float32)
        acc = part + jnp.where(c == 0, 0.0, acc_sc[...])
        acc_sc[...] = acc
        o_ref[...] = acc.astype(o_ref.dtype)

    def block(par, do_a, do_b, do_c, do_d):
        for h in range(hb):
            if do_a:
                s = qk(h)
            if do_b and h > 0:
                pv(h - 1, 1 - par)
            if do_a:
                softmax(h, s, par)
        if do_b:
            pv(hb - 1, 1 - par)
        if do_c:
            outproj(par)
        if do_d:
            qproj(xn_ref, j, (b + 1) % 2)

    @pl.when(t == 0)
    def _():
        for c in range(nj):
            wq_copy(c).start()
        for c in range(nj):
            wo_copy(c).start()
        for c in range(nj):
            wq_copy(c).wait()
            qproj(x0_ref, c, 0)
        block(0, True, False, False, True)

    @pl.when(t == 1)
    def _():
        for c in range(nj):
            wo_copy(c).wait()
        block(1, True, True, False, True)

    @pl.when(jnp.logical_and(jnp.logical_and(t > 1, t < nt), t % 2 == 0))
    def _():
        block(0, True, True, True, True)

    @pl.when(jnp.logical_and(jnp.logical_and(t > 1, t < nt), t % 2 == 1))
    def _():
        block(1, True, True, True, True)

    @pl.when(t == nt)
    def _():
        block(nt % 2, False, True, True, False)

    @pl.when(t == nt + 1)
    def _():
        block((nt + 1) % 2, False, False, True, False)


@jax.jit
def pallas_standalone__gqa_block_cached__near_ridge_kernel(
    x: jax.Array,
    k_cache: jax.Array,
    v_cache: jax.Array,
    wq: jax.Array,
    wo: jax.Array,
):
    B, Sq, D = x.shape
    _, Hkv, Sk, Dh = k_cache.shape
    rep = HQ // Hkv
    hb = HB
    nj = Hkv // hb
    nt = B * nj
    cw = hb * rep * DH
    scale = float(DH) ** -0.5 * 1.4426950408889634
    xt = x.transpose(0, 2, 1)
    wot = wo.T

    def k_map(t):
        tt = jnp.minimum(t, nt - 1)
        return (tt // nj, tt % nj, 0, 0)

    def v_map(t):
        tt = jnp.clip(t - 1, 0, nt - 1)
        return (tt // nj, tt % nj, 0, 0)

    out_t = pl.pallas_call(
        functools.partial(_kernel, hb=hb, rep=rep, nj=nj, nb=B, scale=scale),
        grid=(nt + 2,),
        in_specs=[
            pl.BlockSpec((None, D, Sq), lambda t: (0, 0, 0)),
            pl.BlockSpec((None, D, Sq), lambda t: (jnp.minimum(t // nj + 1, B - 1), 0, 0)),
            pl.BlockSpec((None, hb, Sk, Dh), k_map),
            pl.BlockSpec((None, hb, Sk, Dh), v_map),
            pl.BlockSpec(memory_space=pl.ANY),
            pl.BlockSpec(memory_space=pl.ANY),
        ],
        out_specs=pl.BlockSpec((None, D, Sq), lambda t: (jnp.maximum(t - 2, 0) // nj, 0, 0)),
        out_shape=jax.ShapeDtypeStruct((B, D, Sq), x.dtype),
        scratch_shapes=[
            pltpu.VMEM((nj, D, cw), jnp.bfloat16),
            pltpu.VMEM((nj, D, cw), jnp.bfloat16),
            pltpu.VMEM((2, Hkv, rep * Sq, DH), jnp.bfloat16),
            pltpu.VMEM((hb, rep * Sq, Sk), jnp.bfloat16),
            pltpu.VMEM((hb, rep * Sq, Sk), jnp.bfloat16),
            pltpu.VMEM((hb, rep * Sq, 1), jnp.float32),
            pltpu.VMEM((hb, rep * Sq, 1), jnp.float32),
            pltpu.VMEM((Sq, cw), jnp.bfloat16),
            pltpu.VMEM((Sq, cw), jnp.bfloat16),
            pltpu.VMEM((D, Sq), jnp.float32),
            pltpu.SemaphoreType.DMA((nj,)),
            pltpu.SemaphoreType.DMA((nj,)),
        ],
        compiler_params=pltpu.CompilerParams(
            dimension_semantics=("arbitrary",),
            vmem_limit_bytes=96 * 1024 * 1024,
        ),
    )(xt, xt, k_cache, v_cache, wq, wot)
    return out_t.transpose(0, 2, 1)
```

```python
import functools

import jax
import jax.numpy as jnp
import jax.experimental.pallas as pl
import jax.experimental.pallas.tpu as pltpu

HQ = 32
DH = 128
NJ = 2
RC = 32
WCH = 8


def _kernel(xt_hbm, k_hbm, v_hbm, wq_hbm, wot_hbm, out_hbm,
            x_sc, k0_sc, k1_sc, v0_sc, v1_sc, wq_sc, wo_sc, q_sc,
            p0_sc, p1_sc, r0_sc, r1_sc, a0_sc, a1_sc, acc_sc, o_sc,
            sem_x, sem_k, sem_v, sem_q, sem_o, sem_out,
            *, hb, rep, nb, scale):
    nj = NJ
    sq = x_sc.shape[2]
    d = x_sc.shape[1]
    cw = hb * rep * DH
    nh = hb * rep
    wcw = nj * cw // WCH
    k_sc = (k0_sc, k1_sc)
    v_sc = (v0_sc, v1_sc)
    p_sc = (p0_sc, p1_sc)
    r_sc = (r0_sc, r1_sc)
    a_sc = (a0_sc, a1_sc)

    def x_copy(i):
        if i == 0:
            return pltpu.make_async_copy(xt_hbm.at[pl.ds(0, 2)], x_sc.at[pl.ds(0, 2)], sem_x.at[0])
        return pltpu.make_async_copy(xt_hbm.at[pl.ds(2, nb - 2)], x_sc.at[pl.ds(2, nb - 2)], sem_x.at[1])

    def k_copy(b, j):
        return pltpu.make_async_copy(k_hbm.at[b, pl.ds(j * hb, hb)], k_sc[j], sem_k.at[j])

    def v_copy(b, j):
        return pltpu.make_async_copy(v_hbm.at[b, pl.ds(j * hb, hb)], v_sc[j], sem_v.at[j])

    def wq_copy(c):
        return pltpu.make_async_copy(wq_hbm.at[:, pl.ds(c * wcw, wcw)],
                                     wq_sc.at[:, pl.ds(c * wcw, wcw)], sem_q.at[c])

    def wo_copy(c):
        return pltpu.make_async_copy(wot_hbm.at[:, pl.ds(c * cw, cw)],
                                     wo_sc.at[:, pl.ds(c * cw, cw)], sem_o.at[c])

    def out_copy(b):
        return pltpu.make_async_copy(o_sc, out_hbm.at[b], sem_out.at[0])

    def qproj_cols(xb, slot, col0, ncols):
        q = jax.lax.dot_general(xb, wq_sc[:, col0:col0 + ncols], (((0,), (0,)), ((), ())),
                                preferred_element_type=jnp.float32)
        q = (q * scale).astype(q_sc.dtype)
        for hh in range(ncols // DH):
            h = col0 // DH + hh
            q_sc[slot, h // rep, pl.ds((h % rep) * sq, sq), :] = q[:, hh * DH:(hh + 1) * DH]

    def block(b, j, do_a, do_b, do_c, do_d):
        par = j
        for h in range(hb):
            if do_a:
                s = jax.lax.dot_general(q_sc[b % 2, j * hb + h], k_sc[par][h],
                                        (((1,), (1,)), ((), ())),
                                        preferred_element_type=jnp.float32)
            if do_b and h > 0:
                pv(h - 1, 1 - par)
            if do_a:
                for c in range(0, rep * sq, RC):
                    sc = s[c:c + RC]
                    m = jnp.max(sc, axis=-1, keepdims=True)
                    p = jnp.exp2(sc - m)
                    r_sc[par][h, c:c + RC, :] = 1.0 / jnp.sum(p, axis=-1, keepdims=True)
                    p_sc[par][h, c:c + RC, :] = p.astype(jnp.bfloat16)
        if do_b:
            pv(hb - 1, 1 - par)
        if do_c:
            part = jax.lax.dot_general(wo_sc[:, j * cw:(j + 1) * cw], a_sc[par][...],
                                       (((1,), (1,)), ((), ())),
                                       preferred_element_type=jnp.float32)
            if j == 0:
                acc_sc[...] = part
            else:
                o_sc[...] = (acc_sc[...] + part).astype(o_sc.dtype)
        if do_d:
            qproj_cols(x_sc[jnp.minimum(b + 1, nb - 1)], (b + 1) % 2, j * cw, cw)

    def pv(h, slot):
        o = jnp.dot(p_sc[slot][h], v_sc[slot][h], preferred_element_type=jnp.float32)
        o = (o * r_sc[slot][h]).astype(jnp.bfloat16)
        for rr in range(rep):
            a_sc[slot][:, (h * rep + rr) * DH:(h * rep + rr + 1) * DH] = o[rr * sq:(rr + 1) * sq]

    x_copy(0).start()
    for c in range(WCH):
        wq_copy(c).start()
    k_copy(0, 0).start()
    x_copy(0).wait()
    for c in range(WCH):
        wq_copy(c).wait()
        qproj_cols(x_sc[0], 0, c * wcw, wcw)
    k_copy(0, 1).start()
    v_copy(0, 0).start()
    x_copy(1).start()
    for c in range(nj):
        wo_copy(c).start()
    k_copy(0, 0).wait()
    block(0, 0, True, False, False, True)

    k_copy(1, 0).start()
    v_copy(0, 1).start()
    k_copy(0, 1).wait()
    v_copy(0, 0).wait()
    x_copy(1).wait()
    block(0, 1, True, True, False, True)
    for c in range(nj):
        wo_copy(c).wait()

    def body(b, carry):
        k_copy(b, 1).start()
        v_copy(b, 0).start()
        k_copy(b, 0).wait()
        v_copy(b - 1, 1).wait()
        block(b, 0, True, True, True, True)

        @pl.when(b + 1 < nb)
        def _():
            k_copy(b + 1, 0).start()

        v_copy(b, 1).start()
        k_copy(b, 1).wait()
        v_copy(b, 0).wait()

        @pl.when(b > 1)
        def _():
            out_copy(b - 2).wait()

        block(b, 1, True, True, True, True)
        out_copy(b - 1).start()
        return carry

    jax.lax.fori_loop(1, nb, body, 0)

    v_copy(nb - 1, 1).wait()
    block(nb, 0, False, True, True, False)
    out_copy(nb - 2).wait()
    block(nb, 1, False, False, True, False)
    out_copy(nb - 1).start()
    out_copy(nb - 1).wait()


@jax.jit
def pallas_standalone__gqa_block_cached__near_ridge_kernel(
    x: jax.Array,
    k_cache: jax.Array,
    v_cache: jax.Array,
    wq: jax.Array,
    wo: jax.Array,
):
    B, Sq, D = x.shape
    _, Hkv, Sk, Dh = k_cache.shape
    rep = HQ // Hkv
    hb = Hkv // NJ
    cw = hb * rep * DH
    scale = float(DH) ** -0.5 * 1.4426950408889634
    xt = x.transpose(0, 2, 1)
    wot = wo.T
    bf = jnp.bfloat16

    out_t = pl.pallas_call(
        functools.partial(_kernel, hb=hb, rep=rep, nb=B, scale=scale),
        in_specs=[pl.BlockSpec(memory_space=pl.ANY)] * 5,
        out_specs=pl.BlockSpec(memory_space=pl.ANY),
        out_shape=jax.ShapeDtypeStruct((B, D, Sq), x.dtype),
        scratch_shapes=[
            pltpu.VMEM((B, D, Sq), bf),
            pltpu.VMEM((hb, Sk, Dh), bf), pltpu.VMEM((hb, Sk, Dh), bf),
            pltpu.VMEM((hb, Sk, Dh), bf), pltpu.VMEM((hb, Sk, Dh), bf),
            pltpu.VMEM((D, HQ * DH), bf), pltpu.VMEM((D, HQ * DH), bf),
            pltpu.VMEM((2, Hkv, rep * Sq, DH), bf),
            pltpu.VMEM((hb, rep * Sq, Sk), bf), pltpu.VMEM((hb, rep * Sq, Sk), bf),
            pltpu.VMEM((hb, rep * Sq, 1), jnp.float32), pltpu.VMEM((hb, rep * Sq, 1), jnp.float32),
            pltpu.VMEM((Sq, cw), bf), pltpu.VMEM((Sq, cw), bf),
            pltpu.VMEM((D, Sq), jnp.float32),
            pltpu.VMEM((D, Sq), bf),
            pltpu.SemaphoreType.DMA((2,)),
            pltpu.SemaphoreType.DMA((2,)),
            pltpu.SemaphoreType.DMA((2,)),
            pltpu.SemaphoreType.DMA((WCH,)),
            pltpu.SemaphoreType.DMA((NJ,)),
            pltpu.SemaphoreType.DMA((1,)),
        ],
        compiler_params=pltpu.CompilerParams(
            vmem_limit_bytes=100 * 1024 * 1024,
        ),
    )(xt, k_cache, v_cache, wq, wot)
    return out_t.transpose(0, 2, 1)
```

```python
import functools

import jax
import jax.numpy as jnp
import jax.experimental.pallas as pl
import jax.experimental.pallas.tpu as pltpu

HQ = 32
DH = 128
NJ = 2
RC = 32
WCH = 8


def _kernel(xt_hbm, k_hbm, v_hbm, wq_hbm, wot_hbm, out_hbm,
            x_sc, k0_sc, k1_sc, v0_sc, v1_sc, wq_sc, wo_sc, q_sc,
            p0_sc, p1_sc, r0_sc, r1_sc, a0_sc, a1_sc, acc_sc, o_sc,
            sem_x, sem_k, sem_v, sem_q, sem_o, sem_out,
            *, hb, rep, nb, scale):
    nj = NJ
    sq = x_sc.shape[2]
    d = x_sc.shape[1]
    cw = hb * rep * DH
    nh = hb * rep
    wcw = nj * cw // WCH
    k_sc = (k0_sc, k1_sc)
    v_sc = (v0_sc, v1_sc)
    p_sc = (p0_sc, p1_sc)
    r_sc = (r0_sc, r1_sc)
    a_sc = (a0_sc, a1_sc)

    def x_copy01():
        return pltpu.make_async_copy(xt_hbm.at[pl.ds(0, 2)], x_sc.at[pl.ds(0, 2)], sem_x.at[2])

    def x_copy(bb):
        return pltpu.make_async_copy(xt_hbm.at[bb], x_sc.at[bb], sem_x.at[bb % 2])

    def k_copy(b, j):
        return pltpu.make_async_copy(k_hbm.at[b, pl.ds(j * hb, hb)], k_sc[j], sem_k.at[j])

    def v_copy(b, j):
        return pltpu.make_async_copy(v_hbm.at[b, pl.ds(j * hb, hb)], v_sc[j], sem_v.at[j])

    def wq_copy(c):
        return pltpu.make_async_copy(wq_hbm.at[:, pl.ds(c * wcw, wcw)],
                                     wq_sc.at[:, pl.ds(c * wcw, wcw)], sem_q.at[c])

    def wo_copy(c):
        return pltpu.make_async_copy(wot_hbm.at[:, pl.ds(c * cw, cw)],
                                     wo_sc.at[:, pl.ds(c * cw, cw)], sem_o.at[c])

    def out_copy(b):
        return pltpu.make_async_copy(o_sc, out_hbm.at[b], sem_out.at[0])

    def qproj_cols(xb, slot, col0, ncols):
        q = jax.lax.dot_general(xb, wq_sc[:, col0:col0 + ncols], (((0,), (0,)), ((), ())),
                                preferred_element_type=jnp.float32)
        q = (q * scale).astype(q_sc.dtype)
        for hh in range(ncols // DH):
            h = col0 // DH + hh
            q_sc[slot, h // rep, pl.ds((h % rep) * sq, sq), :] = q[:, hh * DH:(hh + 1) * DH]

    def block(b, j, do_a, do_b, do_c, do_d):
        par = j
        for h in range(hb):
            if do_a:
                s = jax.lax.dot_general(q_sc[b % 2, j * hb + h], k_sc[par][h],
                                        (((1,), (1,)), ((), ())),
                                        preferred_element_type=jnp.float32)
            if do_b and h > 0:
                pv(h - 1, 1 - par)
            if do_a:
                for c in range(0, rep * sq, RC):
                    sc = s[c:c + RC]
                    m = jnp.max(sc, axis=-1, keepdims=True)
                    p = jnp.exp2(sc - m)
                    r_sc[par][h, c:c + RC, :] = 1.0 / jnp.sum(p, axis=-1, keepdims=True)
                    p_sc[par][h, c:c + RC, :] = p.astype(jnp.bfloat16)
        if do_b:
            pv(hb - 1, 1 - par)
        if do_c:
            part = jax.lax.dot_general(wo_sc[:, j * cw:(j + 1) * cw], a_sc[par][...],
                                       (((1,), (1,)), ((), ())),
                                       preferred_element_type=jnp.float32)
            if j == 0:
                acc_sc[...] = part
            else:
                o_sc[...] = (acc_sc[...] + part).astype(o_sc.dtype)
        if do_d:
            qproj_cols(x_sc[jnp.minimum(b + 1, nb - 1)], (b + 1) % 2, j * cw, cw)

    def pv(h, slot):
        o = jnp.dot(p_sc[slot][h], v_sc[slot][h], preferred_element_type=jnp.float32)
        o = (o * r_sc[slot][h]).astype(jnp.bfloat16)
        for rr in range(rep):
            a_sc[slot][:, (h * rep + rr) * DH:(h * rep + rr + 1) * DH] = o[rr * sq:(rr + 1) * sq]

    x_copy01().start()
    for c in range(WCH):
        wq_copy(c).start()
    k_copy(0, 0).start()
    x_copy01().wait()
    for c in range(WCH):
        wq_copy(c).wait()
        if c == WCH // 2:
            k_copy(0, 1).start()
            v_copy(0, 0).start()
        qproj_cols(x_sc[0], 0, c * wcw, wcw)
    k_copy(0, 0).wait()
    block(0, 0, True, False, False, True)

    k_copy(1, 0).start()
    v_copy(0, 1).start()
    wo_copy(0).start()
    x_copy(2).start()
    k_copy(0, 1).wait()
    v_copy(0, 0).wait()
    block(0, 1, True, True, False, True)

    def body(b, carry):
        k_copy(b, 1).start()
        v_copy(b, 0).start()

        @pl.when(b == 1)
        def _():
            wo_copy(1).start()
            wo_copy(0).wait()

        @pl.when(b + 1 < nb)
        def _():
            x_copy(b + 1).wait()

        @pl.when(b + 2 < nb)
        def _():
            x_copy(b + 2).start()

        k_copy(b, 0).wait()
        v_copy(b - 1, 1).wait()
        block(b, 0, True, True, True, True)

        @pl.when(b + 1 < nb)
        def _():
            k_copy(b + 1, 0).start()

        v_copy(b, 1).start()
        k_copy(b, 1).wait()
        v_copy(b, 0).wait()

        @pl.when(b == 1)
        def _():
            wo_copy(1).wait()

        @pl.when(b > 1)
        def _():
            out_copy(b - 2).wait()

        block(b, 1, True, True, True, True)
        out_copy(b - 1).start()
        return carry

    jax.lax.fori_loop(1, nb, body, 0)

    v_copy(nb - 1, 1).wait()
    block(nb, 0, False, True, True, False)
    out_copy(nb - 2).wait()
    block(nb, 1, False, False, True, False)
    out_copy(nb - 1).start()
    out_copy(nb - 1).wait()


@jax.jit
def pallas_standalone__gqa_block_cached__near_ridge_kernel(
    x: jax.Array,
    k_cache: jax.Array,
    v_cache: jax.Array,
    wq: jax.Array,
    wo: jax.Array,
):
    B, Sq, D = x.shape
    _, Hkv, Sk, Dh = k_cache.shape
    rep = HQ // Hkv
    hb = Hkv // NJ
    cw = hb * rep * DH
    scale = float(DH) ** -0.5 * 1.4426950408889634
    xt = x.transpose(0, 2, 1)
    wot = wo.T
    bf = jnp.bfloat16

    out_t = pl.pallas_call(
        functools.partial(_kernel, hb=hb, rep=rep, nb=B, scale=scale),
        in_specs=[pl.BlockSpec(memory_space=pl.ANY)] * 5,
        out_specs=pl.BlockSpec(memory_space=pl.ANY),
        out_shape=jax.ShapeDtypeStruct((B, D, Sq), x.dtype),
        scratch_shapes=[
            pltpu.VMEM((B, D, Sq), bf),
            pltpu.VMEM((hb, Sk, Dh), bf), pltpu.VMEM((hb, Sk, Dh), bf),
            pltpu.VMEM((hb, Sk, Dh), bf), pltpu.VMEM((hb, Sk, Dh), bf),
            pltpu.VMEM((D, HQ * DH), bf), pltpu.VMEM((D, HQ * DH), bf),
            pltpu.VMEM((2, Hkv, rep * Sq, DH), bf),
            pltpu.VMEM((hb, rep * Sq, Sk), bf), pltpu.VMEM((hb, rep * Sq, Sk), bf),
            pltpu.VMEM((hb, rep * Sq, 1), jnp.float32), pltpu.VMEM((hb, rep * Sq, 1), jnp.float32),
            pltpu.VMEM((Sq, cw), bf), pltpu.VMEM((Sq, cw), bf),
            pltpu.VMEM((D, Sq), jnp.float32),
            pltpu.VMEM((D, Sq), bf),
            pltpu.SemaphoreType.DMA((3,)),
            pltpu.SemaphoreType.DMA((2,)),
            pltpu.SemaphoreType.DMA((2,)),
            pltpu.SemaphoreType.DMA((WCH,)),
            pltpu.SemaphoreType.DMA((NJ,)),
            pltpu.SemaphoreType.DMA((1,)),
        ],
        compiler_params=pltpu.CompilerParams(
            vmem_limit_bytes=100 * 1024 * 1024,
        ),
    )(xt, k_cache, v_cache, wq, wot)
    return out_t.transpose(0, 2, 1)
```
